```python
import os as _os
_os.environ.setdefault("JAX_PLATFORMS", "cpu")
import jax
import jax.numpy as jnp

def _softmax(x, axis=-1):
    return jax.nn.softmax(x, axis=axis)
def _gelu(x):
    return jax.nn.gelu(x, approximate=True)
def _silu(x):
    return jax.nn.silu(x)
def _sigmoid(x):
    return jax.nn.sigmoid(x)
def _layernorm(x, axis=-1, eps=1e-5):
    m = jnp.mean(x, axis=axis, keepdims=True)
    v = jnp.var(x, axis=axis, keepdims=True)
    return (x - m) / jnp.sqrt(v + eps)
def _scatter_add(tgt, idx, src, axis=0):
    return tgt.at[idx].add(src)
def _segment_sum(src, seg, n):
    return jax.ops.segment_sum(src, seg, n)
class _Rng:
    def __init__(self, key):
        self._k = key
    def _next(self):
        self._k, sub = jax.random.split(self._k)
        return sub
    def normal(self, shape):
        return jax.random.normal(self._next(), shape, dtype=jnp.bfloat16)
    def randint(self, lo, hi, shape):
        return jax.random.randint(self._next(), shape, lo, hi, dtype=jnp.int32)
    def uniform(self, shape, lo=0.0, hi=1.0):
        return jax.random.uniform(self._next(), shape, jnp.bfloat16, lo, hi)
    def permutation(self, n):
        return jax.random.permutation(self._next(), n)


kernel_name = 'interleave_layers__grouped_kv_mqa__dense_activation_relu__prompt'

def setup_inputs():
    _rng = _Rng(jax.random.key(int.from_bytes(__import__("os").urandom(4), "little")))
    _w = (lambda a: (lambda t: t.astype(jnp.bfloat16) if jnp.issubdtype(t.dtype, jnp.floating) else t)(jnp.asarray(a)))
    def _A_setup():
        B, S, D, H = 1, 2048, 448, 16
        Dh = D // H
        return {
            "x": _w((lambda *s: _rng.normal(s) * 0.05)(B, S, D)),
            "wq": _w((lambda *s: _rng.normal(s) * 0.05)(D, H * Dh)),
            "wk": _w((lambda *s: _rng.normal(s) * 0.05)(D, Dh)),
            "wv": _w((lambda *s: _rng.normal(s) * 0.05)(D, Dh)),
            "wo": _w((lambda *s: _rng.normal(s) * 0.05)(H * Dh, D)),
        }
    _A_in = _A_setup()

    def _B_setup():
        B, S, D, Dff = 1, 2048, 448, 1792
        return {
            "x": _w((lambda *s: _rng.normal(s) * 0.05)(B, S, D)),
            "w1": _w((lambda *s: _rng.normal(s) * 0.05)(D, Dff)),
            "w2": _w((lambda *s: _rng.normal(s) * 0.05)(Dff, D)),
        }
    _B_in = _B_setup()

    return {
        "A_x": _A_in["x"],
        "A_wq": _A_in["wq"],
        "A_wk": _A_in["wk"],
        "A_wv": _A_in["wv"],
        "A_wo": _A_in["wo"],
        "B_x": _B_in["x"],
        "B_w1": _B_in["w1"],
        "B_w2": _B_in["w2"],
    }

def reference(A_x, A_wq, A_wk, A_wv, A_wo, B_x, B_w1, B_w2):
    def _A_ref(x, wq, wk, wv, wo):
        B, S, D = x.shape
        H = 16
        Dh = D // H
        q = (lambda x, *d: x.transpose(*d))((x @ wq).reshape(B, S, H, Dh), 0, 2, 1, 3)
        k = x @ wk
        v = x @ wv
        scores = jnp.einsum("bhqd,bkd->bhqk", q, k) * (Dh ** -0.5)
        p = _softmax(scores, axis=-1)
        o = jnp.einsum("bhqk,bkd->bhqd", p, v)
        return (lambda x, *d: x.transpose(*d))(o, 0, 2, 1, 3).reshape(B, S, H * Dh) @ wo

    def _B_ref(x, w1, w2):
        h = jnp.einsum("bsd,df->bsf", x, w1)
        zero = jnp.zeros_like(h)
        h = jnp.maximum(h, zero)
        return jnp.einsum("bsf,fd->bsd", h, w2)

    x = A_x
    x = x + _A_ref(_layernorm(x, axis=-1), A_wq, A_wk, A_wv, A_wo)
    x = x + _B_ref(_layernorm(x, axis=-1), B_w1, B_w2)
    x = x + _A_ref(_layernorm(x, axis=-1), A_wq, A_wk, A_wv, A_wo)
    x = x + _B_ref(_layernorm(x, axis=-1), B_w1, B_w2)
    return x
```

```python
import functools, math
import jax, jax.numpy as jnp
from jax import lax
from jax.experimental import pallas as pl
from jax.experimental.pallas import tpu as pltpu

S, D, H, DH, HP, F = 2048, 448, 16, 28, 32, 1792
EPS = 1e-5
bf16, f32, u32 = jnp.bfloat16, jnp.float32, jnp.uint32
QSCALE = (DH ** -0.5) * math.log2(math.e)
NT = (((1,), (1,)), ((), ()))

def _ln_t(x):
    mean = jnp.sum(x, axis=0, keepdims=True) * (1.0 / D)
    xc = x - mean
    var = jnp.sum(xc * xc, axis=0, keepdims=True) * (1.0 / D)
    return (xc * lax.rsqrt(var + EPS)).astype(bf16)

def _dot(a, b):
    return jnp.dot(a, b, preferred_element_type=f32)

def _dot_nt(a, b):
    return lax.dot_general(a, b, NT, preferred_element_type=f32)

def _sel(rows, cols, fn):
    r = lax.broadcasted_iota(jnp.int32, (rows, cols), 0)
    c = lax.broadcasted_iota(jnp.int32, (rows, cols), 1)
    return jnp.where(fn(r, c), 1.0, 0.0).astype(bf16)

def make_kernel(T=512, CK=128, CB=256, skip=()):
    NB = S // T
    NJ = NB * H

    def kernel(xt_hbm, wq_hbm, wkt_hbm, wvt_hbm, wo_hbm, w1_hbm, w2t_hbm, o_hbm,
               xin_ref, wq_ref, wkt_ref, wvt_ref, wo_ref, w1_ref, w2t_ref, xout_ref,
               xt_ref, qt_ref, ot_ref, k_ref, vt_ref, s_ref, p0_ref, p1_ref, ht_ref,
               wqt_ref, wkvt_ref, wot_ref, w1t_ref, sem_in, sem_w, sem_out):
        x_cp = [pltpu.make_async_copy(xt_hbm.at[:, b * T:(b + 1) * T], xin_ref.at[b], sem_in.at[b]) for b in range(NB)]
        w_cp = [pltpu.make_async_copy(src, dst, sem_w.at[i]) for i, (src, dst) in enumerate(
            [(wq_hbm, wq_ref), (wkt_hbm, wkt_ref), (wvt_hbm, wvt_ref), (wo_hbm, wo_ref), (w1_hbm, w1_ref), (w2t_hbm, w2t_ref)])]
        w_cp[0].start(); x_cp[0].start(); w_cp[1].start(); w_cp[2].start()
        for b in range(1, NB):
            x_cp[b].start()
        w_cp[3].start(); w_cp[4].start(); w_cp[5].start()

        w_cp[0].wait()
        G = 4 * DH
        for g in range(4):
            lo = (g * G) // 128 * 128
            hi = min(-(-((g + 1) * G) // 128) * 128, D)
            e = _sel(128, hi - lo, lambda r, c: ((r % HP) < DH) & (c + lo == g * G + (r // HP) * DH + (r % HP)))
            wqt_ref[g * 128:(g + 1) * 128, :] = _dot_nt(e, wq_ref[:, lo:hi]).astype(bf16)
        w_cp[1].wait(); w_cp[2].wait()
        wkvt_ref[...] = jnp.zeros(wkvt_ref.shape, bf16)
        wkvt_ref[0:DH, :] = wkt_ref[...]
        wkvt_ref[HP:HP + DH, :] = wvt_ref[...]

        def qkv(b, x):
            ln = _ln_t(x)
            qt_ref[b] = (_dot(wqt_ref[...], ln) * QSCALE).astype(bf16)
            kv = _dot(wkvt_ref[...], ln)
            k_ref[pl.ds(pl.multiple_of(b * T, T), T), :] = kv[0:HP].T.astype(bf16)
            row = lax.broadcasted_iota(jnp.int32, (HP, T), 0)
            vt_ref[b] = jnp.where(row == DH, 1.0, kv[HP:2 * HP]).astype(bf16)

        for b in range(NB):
            x_cp[b].wait()
            x = xin_ref[b].astype(f32)
            xt_ref[b] = x
            qkv(b, x)

        def prep_post_weights():
            w_cp[3].wait(); w_cp[4].wait(); w_cp[5].wait()
            eye128 = _sel(128, 128, lambda r, c: r == c)
            for n0 in range(0, D, 128):
                n1 = min(n0 + 128, D)
                wt = _dot_nt(eye128[0:n1 - n0, 0:n1 - n0], wo_ref[:, n0:n1]).astype(bf16)
                for g in range(4):
                    lo = (g * G) // 128 * 128
                    hi = min(-(-((g + 1) * G) // 128) * 128, D)
                    e = _sel(hi - lo, 128, lambda r, c: ((c % HP) < DH) & (r + lo == g * G + (c // HP) * DH + (c % HP)))
                    wot_ref[n0:n1, g * 128:(g + 1) * 128] = _dot(wt[:, lo:hi], e).astype(bf16)
            for j in range(F // 128):
                w1t_ref[j * 128:(j + 1) * 128, :] = _dot_nt(eye128, w1_ref[:, j * 128:(j + 1) * 128]).astype(bf16)

        def step(ja, jb_p_ref, mb, jc, pc_ref):
            if jb_p_ref is not None:
                for c0 in range(0, S, CB):
                    p = jnp.exp2(s_ref[c0:c0 + CB, :] - mb).astype(bf16)
                    jb_p_ref[c0 // 2:(c0 + CB) // 2, :] = pltpu.bitcast(p, u32)
            m = None
            if ja is not None:
                q = qt_ref[ja // H, pl.ds(pl.multiple_of((ja % H) * HP, HP), HP), :]
                s = _dot(k_ref[...], q)
                s_ref[...] = s
                m = jnp.max(s, axis=0, keepdims=True)
            if jc is not None:
                acc = jnp.zeros((HP, T), f32)
                for c0 in range(0, S, CK):
                    p = pltpu.bitcast(pc_ref[c0 // 2:(c0 + CK) // 2, :], bf16)
                    kb, off = c0 // T, c0 % T
                    acc = acc + _dot(vt_ref[kb, :, off:off + CK], p)
                o = acc * (1.0 / acc[DH:DH + 1, :])
                ot_ref[jc // H, pl.ds(pl.multiple_of((jc % H) * HP, HP), HP), :] = o.astype(bf16)
            return m

        def attention():
            m0 = step(0, None, None, None, None)
            m1 = step(1, p0_ref, m0, None, None)
            def body(jj, m):
                j = 2 * jj
                m2 = step(j + 2, p1_ref, m, j, p0_ref)
                m3 = step(j + 3, p0_ref, m2, j + 1, p1_ref)
                return m3
            m = lax.fori_loop(0, NJ // 2 - 1, body, m1)
            step(None, p1_ref, m, NJ - 2, p0_ref)
            step(None, None, None, NJ - 1, p1_ref)

        def out_cp(b):
            return pltpu.make_async_copy(xout_ref.at[b], o_hbm.at[:, pl.ds(pl.multiple_of(b * T, T), T)], sem_out.at[b])

        def post(layer):
            def body(b, carry):
                x = xt_ref[b] + _dot(wot_ref[...], ot_ref[b])
                ln = _ln_t(x)
                ht_ref[...] = jnp.maximum(_dot(w1t_ref[...], ln), 0.0).astype(bf16)
                x = x + _dot(w2t_ref[...], ht_ref[...])
                if layer == 0:
                    xt_ref[b] = x
                    qkv(b, x)
                else:
                    xout_ref[b] = x.astype(bf16)
                    out_cp(b).start()
                return carry
            lax.fori_loop(0, NB, body, 0)

        if 'attn' not in skip: attention()
        prep_post_weights()
        if 'post' not in skip: post(0)
        if 'attn' not in skip: attention()
        post(1)
        for b in range(NB):
            out_cp(b).wait()

    scratch = [
        pltpu.VMEM((NB, D, T), bf16),
        pltpu.VMEM((D, D), bf16),
        pltpu.VMEM((DH, D), bf16),
        pltpu.VMEM((DH, D), bf16),
        pltpu.VMEM((D, D), bf16),
        pltpu.VMEM((D, F), bf16),
        pltpu.VMEM((D, F), bf16),
        pltpu.VMEM((NB, D, T), bf16),
        pltpu.VMEM((NB, D, T), f32),
        pltpu.VMEM((NB, H * HP, T), bf16),
        pltpu.VMEM((NB, H * HP, T), bf16),
        pltpu.VMEM((S, HP), bf16),
        pltpu.VMEM((NB, HP, T), bf16),
        pltpu.VMEM((S, T), f32),
        pltpu.VMEM((S // 2, T), u32),
        pltpu.VMEM((S // 2, T), u32),
        pltpu.VMEM((F, T), bf16),
        pltpu.VMEM((H * HP, D), bf16),
        pltpu.VMEM((2 * HP, D), bf16),
        pltpu.VMEM((D, H * HP), bf16),
        pltpu.VMEM((F, D), bf16),
        pltpu.SemaphoreType.DMA((NB,)),
        pltpu.SemaphoreType.DMA((6,)),
        pltpu.SemaphoreType.DMA((NB,)),
    ]
    return kernel, scratch


_KERNEL, _SCRATCH = make_kernel()


@jax.jit
def pallas_interleave_layers__grouped_kv_mqa__dense_activation_relu__prompt_kernel(
    A_x: jax.Array,
    A_wq: jax.Array,
    A_wk: jax.Array,
    A_wv: jax.Array,
    A_wo: jax.Array,
    B_x: jax.Array,
    B_w1: jax.Array,
    B_w2: jax.Array,
):
    del B_x
    out = pl.pallas_call(
        _KERNEL,
        out_shape=jax.ShapeDtypeStruct((D, S), bf16),
        in_specs=[pl.BlockSpec(memory_space=pl.ANY)] * 7,
        out_specs=pl.BlockSpec(memory_space=pl.ANY),
        scratch_shapes=_SCRATCH,
        compiler_params=pltpu.CompilerParams(vmem_limit_bytes=100 * 1024 * 1024),
    )(A_x.reshape(S, D).T, A_wq, A_wk.T, A_wv.T, A_wo, B_w1, B_w2.T)
    return out.T.reshape(1, S, D)
```

```python
import functools, math
import jax, jax.numpy as jnp
from jax import lax
from jax.experimental import pallas as pl
from jax.experimental.pallas import tpu as pltpu

S, D, H, DH, HP, F = 2048, 448, 16, 28, 32, 1792
EPS = 1e-5
bf16, f32, u32 = jnp.bfloat16, jnp.float32, jnp.uint32
QSCALE = (DH ** -0.5) * math.log2(math.e)
NT = (((1,), (1,)), ((), ()))
SAFE_BOUND = 45.0

def _ln_t(x):
    mean = jnp.sum(x, axis=0, keepdims=True) * (1.0 / D)
    xc = x - mean
    var = jnp.sum(xc * xc, axis=0, keepdims=True) * (1.0 / D)
    return (xc * lax.rsqrt(var + EPS)).astype(bf16)

def _dot(a, b):
    return jnp.dot(a, b, preferred_element_type=f32)

def _dot_nt(a, b):
    return lax.dot_general(a, b, NT, preferred_element_type=f32)

def _sel(rows, cols, fn):
    r = lax.broadcasted_iota(jnp.int32, (rows, cols), 0)
    c = lax.broadcasted_iota(jnp.int32, (rows, cols), 1)
    return jnp.where(fn(r, c), 1.0, 0.0).astype(bf16)

def make_kernel(T=512, CK=128, CB=256, skip=(), NVK=0, KT=4, FA=0.7, force=None):
    NB = S // T
    NJ = NB * H
    SM = S - NVK
    NL = T // 128
    NG = NVK // (8 * KT) if NVK else 0
    NCH = NL * NG

    def kernel(xt_hbm, wq_hbm, wkt_hbm, wvt_hbm, wo_hbm, w1_hbm, w2t_hbm, o_hbm,
               xin_ref, wq_ref, wkt_ref, wvt_ref, wo_ref, w1_ref, w2t_ref, xout_ref,
               xt_ref, qt_ref, ot_ref, k_ref, vt_ref, s_ref, p0_ref, p1_ref, ht_ref,
               wqt_ref, wkvt_ref, wot_ref, w1t_ref, kb_ref, qf_ref, nrm_ref, false_ref, sem_in, sem_w, sem_out):
        x_cp = [pltpu.make_async_copy(xt_hbm.at[:, b * T:(b + 1) * T], xin_ref.at[b], sem_in.at[b]) for b in range(NB)]
        w_cp = [pltpu.make_async_copy(src, dst, sem_w.at[i]) for i, (src, dst) in enumerate(
            [(wq_hbm, wq_ref), (wkt_hbm, wkt_ref), (wvt_hbm, wvt_ref), (wo_hbm, wo_ref), (w1_hbm, w1_ref), (w2t_hbm, w2t_ref)])]
        false_ref[...] = jnp.zeros((8, 128), jnp.int32)
        w_cp[0].start(); x_cp[0].start(); w_cp[1].start(); w_cp[2].start()

        G = 4 * DH
        eye128 = _sel(128, 128, lambda r, c: r == c)
        w_cp[0].wait()
        for b in range(1, NB):
            x_cp[b].start()
        for n0 in range(0, D, 128):
            n1 = min(n0 + 128, D)
            wqt_ref[n0:n1, :] = _dot_nt(eye128[0:n1 - n0, 0:n1 - n0], wq_ref[:, n0:n1]).astype(bf16)
        w_cp[1].wait(); w_cp[2].wait()
        wqt_ref[D:D + 2 * HP, :] = jnp.zeros((2 * HP, D), bf16)
        wqt_ref[D:D + DH, :] = wkt_ref[...]
        wqt_ref[D + HP:D + HP + DH, :] = wvt_ref[...]

        def qkv(b, x):
            ln = _ln_t(x)
            r = _dot(wqt_ref[...], ln)
            q = (r[0:D] * QSCALE).astype(bf16).astype(f32)
            heads, qns = [], []
            zpad = jnp.zeros((HP - DH - 1, T), f32)
            for h in range(H):
                qh = q[h * DH:(h + 1) * DH]
                qn = jnp.sqrt(jnp.sum(qh * qh, axis=0, keepdims=True))
                qns.append(qn)
                qt_ref[b, h * HP:(h + 1) * HP, :] = jnp.concatenate([qh, qn, zpad], axis=0).astype(bf16)
            qmax = qns[0]
            for qn in qns[1:]:
                qmax = jnp.maximum(qmax, qn)
            kb16 = r[D:D + HP].astype(bf16).astype(f32)
            kn2 = jnp.sum(kb16 * kb16, axis=0, keepdims=True)
            nrm_ref[b, 0:1, :] = qmax
            nrm_ref[b, 1:2, :] = kn2
            k_ref[pl.ds(pl.multiple_of(b * (T // 2), T // 2), T // 2), :] = pltpu.bitcast(kb16.T.astype(bf16), u32)
            row = lax.broadcasted_iota(jnp.int32, (HP, T), 0)
            vt_ref[b] = jnp.where(row == DH, 1.0, r[D + HP:D + 2 * HP]).astype(bf16)

        for b in range(NB):
            if b == 0:
                x_cp[0].wait()
            if b == 1:
                for bb in range(1, NB):
                    x_cp[bb].wait()
                w_cp[3].start(); w_cp[4].start(); w_cp[5].start()
            x = xin_ref[b].astype(f32)
            xt_ref[b] = x
            qkv(b, x)

        def prep_post_weights():
            w_cp[3].wait(); w_cp[4].wait(); w_cp[5].wait()
            for n0 in range(0, D, 128):
                n1 = min(n0 + 128, D)
                wt = _dot_nt(eye128[0:n1 - n0, 0:n1 - n0], wo_ref[:, n0:n1]).astype(bf16)
                for g in range(4):
                    lo = (g * G) // 128 * 128
                    hi = min(-(-((g + 1) * G) // 128) * 128, D)
                    e = _sel(hi - lo, 128, lambda r, c: ((c % HP) < DH) & (r + lo == g * G + (c // HP) * DH + (c % HP)))
                    wot_ref[n0:n1, g * 128:(g + 1) * 128] = _dot(wt[:, lo:hi], e).astype(bf16)
            for j in range(F // 128):
                w1t_ref[j * 128:(j + 1) * 128, :] = _dot_nt(eye128, w1_ref[:, j * 128:(j + 1) * 128]).astype(bf16)

        def load_q(j):
            return qt_ref[j // H, pl.ds(pl.multiple_of((j % H) * HP, HP), HP), :]

        def stage_c(jc, pc_ref, hook=None):
            acc = jnp.zeros((HP, T), f32)
            for c0 in range(0, S, CK):
                p = pltpu.bitcast(pc_ref[c0 // 2:(c0 + CK) // 2, :], bf16)
                kb, off = c0 // T, c0 % T
                part = _dot(vt_ref[kb, :, off:off + CK], p)
                if hook is not None:
                    hook(c0, part)
                acc = acc + part
            o = acc * (1.0 / acc[DH:DH + 1, :])
            ot_ref[jc // H, pl.ds(pl.multiple_of((jc % H) * HP, HP), HP), :] = o.astype(bf16)

        def step_safe(ja, jb_p_ref, mb, jc, pc_ref):
            if jb_p_ref is not None:
                for c0 in range(0, S, CB):
                    p = jnp.exp2(s_ref[c0:c0 + CB, :] - mb).astype(bf16)
                    jb_p_ref[c0 // 2:(c0 + CB) // 2, :] = pltpu.bitcast(p, u32)
            m = None
            if ja is not None:
                q = load_q(ja)
                row = lax.broadcasted_iota(jnp.int32, (HP, T), 0)
                q = jnp.where(row == DH, jnp.zeros_like(q), q)
                s = _dot(pltpu.bitcast(k_ref[...], bf16), q)
                s_ref[...] = s
                m = jnp.max(s, axis=0, keepdims=True)
            if jc is not None:
                stage_c(jc, pc_ref)
            return m

        def attention_safe():
            m0 = step_safe(0, None, None, None, None)
            m1 = step_safe(1, p0_ref, m0, None, None)
            def body(jj, m):
                j = 2 * jj
                m2 = step_safe(j + 2, p1_ref, m, j, p0_ref)
                m3 = step_safe(j + 3, p0_ref, m2, j + 1, p1_ref)
                return m3
            m = lax.fori_loop(0, NJ // 2 - 1, body, m1)
            step_safe(None, p1_ref, m, NJ - 2, p0_ref)
            step_safe(None, None, None, NJ - 1, p1_ref)

        def step_fast(ja, pa_ref, jc, pc_ref, vpu=True):
            chains = []
            if ja is not None:
                q = load_q(ja)
                sm = SM if vpu else S
                s = _dot(pltpu.bitcast(k_ref[0:sm // 2, :], bf16), q)
                pa_ref[0:sm // 2, :] = pltpu.bitcast(jnp.exp2(s).astype(bf16), u32)
                if NVK and vpu:
                    qf = q.astype(f32)
                    row = lax.broadcasted_iota(jnp.int32, (HP, T), 0)
                    qf_ref[...] = jnp.where(row == DH, qf * kb_ref[DH, 0:1, 0:1], qf)
                    false = false_ref[...] != 0

                    def chain(ci, tokens):
                        l, g = ci // NG, ci % NG
                        acc = None
                        for i, d in enumerate([DH] + list(range(DH))):
                            qr = jnp.broadcast_to(qf_ref[d:d + 1, l * 128:(l + 1) * 128], (8, 128))
                            tok = tokens(i)
                            if tok is not None:
                                qr = jnp.where(false, tok, qr)
                            qr = jnp.concatenate([qr] * KT, axis=0)
                            if d == DH:
                                acc = qr
                            else:
                                acc = acc + kb_ref[d, g * 8 * KT:(g + 1) * 8 * KT, :] * qr
                        r0 = SM + g * 8 * KT
                        pa_ref[r0 // 2:(r0 + 8 * KT) // 2, l * 128:(l + 1) * 128] = pltpu.bitcast(jnp.exp2(acc).astype(bf16), u32)

                    NA = NCH if jc is None else int(round(NCH * FA))
                    for ci in range(NA):
                        def tokens(i, ci=ci):
                            n = ci * (DH + 1) + i
                            r = (n * (SM // 8)) // (NA * (DH + 1))
                            l = ci // NG
                            return s[r * 8:(r + 1) * 8, l * 128:(l + 1) * 128]
                        chain(ci, tokens)
                    chains = list(range(NA, NCH))
            hook = None
            if chains:
                nsteps = len(chains) * (DH + 1)
                ntile = S // CK
                toks = {}
                def hook(c0, pu):
                    toks[c0 // CK] = pu
            if jc is not None:
                stage_c(jc, pc_ref, hook)
                for k, ci in enumerate(chains):
                    def tokens(i, k=k):
                        n = k * (DH + 1) + i
                        pos = (n * ntile * (HP // 8) * NL) // nsteps
                        t, rem = pos // ((HP // 8) * NL), pos % ((HP // 8) * NL)
                        r, l = rem // NL, rem % NL
                        return toks[t][r * 8:(r + 1) * 8, l * 128:(l + 1) * 128]
                    chain(ci, tokens)

        def attention_fast(kmax):
            col = lax.broadcasted_iota(jnp.int32, (S // 2, HP), 1)
            nk = jnp.full((16, HP), -kmax, f32).astype(bf16)
            nk_u = pltpu.bitcast(nk, u32)[0:1, :]
            k_ref[...] = jnp.where(col == DH, nk_u, k_ref[...])
            if NVK:
                kf = pltpu.bitcast(k_ref[SM // 2:S // 2, :], bf16).astype(f32)
                for d in range(DH + 1):
                    kb_ref[d] = jnp.broadcast_to(kf[:, d:d + 1], (NVK, 128))
            step_fast(0, p0_ref, None, None, vpu=False)
            def body(jj, c):
                j = 2 * jj
                step_fast(j + 1, p1_ref, j, p0_ref)
                step_fast(j + 2, p0_ref, j + 1, p1_ref)
                return c
            lax.fori_loop(0, NJ // 2 - 1, body, 0)
            step_fast(NJ - 1, p1_ref, NJ - 2, p0_ref)
            step_fast(None, None, NJ - 1, p1_ref)

        def attention():
            nr = nrm_ref[...]
            qmax = jnp.max(nr[:, 0:1, :])
            kmax = jnp.sqrt(jnp.max(nr[:, 1:2, :])) * 1.01
            safe = qmax * kmax <= SAFE_BOUND
            if force == 'fast':
                attention_fast(kmax)
            elif force == 'safe':
                attention_safe()
            else:
                @pl.when(safe)
                def _():
                    attention_fast(kmax)
                @pl.when(jnp.logical_not(safe))
                def _():
                    attention_safe()

        def out_cp(b):
            return pltpu.make_async_copy(xout_ref.at[b], o_hbm.at[:, pl.ds(pl.multiple_of(b * T, T), T)], sem_out.at[b])

        def post(layer):
            def body(b, carry):
                x = xt_ref[b] + _dot(wot_ref[...], ot_ref[b])
                ln = _ln_t(x)
                ht_ref[...] = jnp.maximum(_dot(w1t_ref[...], ln), 0.0).astype(bf16)
                x = x + _dot(w2t_ref[...], ht_ref[...])
                if layer == 0:
                    xt_ref[b] = x
                    qkv(b, x)
                else:
                    xout_ref[b] = x.astype(bf16)
                    out_cp(b).start()
                return carry
            lax.fori_loop(0, NB, body, 0)

        if 'attn' not in skip: attention()
        prep_post_weights()
        if 'post' not in skip: post(0)
        if 'attn' not in skip: attention()
        post(1)
        for b in range(NB):
            out_cp(b).wait()

    scratch = [
        pltpu.VMEM((NB, D, T), bf16),
        pltpu.VMEM((D, D), bf16),
        pltpu.VMEM((DH, D), bf16),
        pltpu.VMEM((DH, D), bf16),
        pltpu.VMEM((D, D), bf16),
        pltpu.VMEM((D, F), bf16),
        pltpu.VMEM((D, F), bf16),
        pltpu.VMEM((NB, D, T), bf16),
        pltpu.VMEM((NB, D, T), f32),
        pltpu.VMEM((NB, H * HP, T), bf16),
        pltpu.VMEM((NB, H * HP, T), bf16),
        pltpu.VMEM((S // 2, HP), u32),
        pltpu.VMEM((NB, HP, T), bf16),
        pltpu.VMEM((S, T), f32),
        pltpu.VMEM((S // 2, T), u32),
        pltpu.VMEM((S // 2, T), u32),
        pltpu.VMEM((F, T), bf16),
        pltpu.VMEM((D + 2 * HP, D), bf16),
        pltpu.VMEM((2 * HP, D), bf16),
        pltpu.VMEM((D, H * HP), bf16),
        pltpu.VMEM((F, D), bf16),
        pltpu.VMEM((DH + 1, max(NVK, 8), 128), f32),
        pltpu.VMEM((HP, T), f32),
        pltpu.VMEM((NB, 2, T), f32),
        pltpu.VMEM((8, 128), jnp.int32),
        pltpu.SemaphoreType.DMA((NB,)),
        pltpu.SemaphoreType.DMA((6,)),
        pltpu.SemaphoreType.DMA((NB,)),
    ]
    return kernel, scratch


_KERNEL, _SCRATCH = make_kernel(NVK=192, FA=0.84, KT=8)


@jax.jit
def pallas_interleave_layers__grouped_kv_mqa__dense_activation_relu__prompt_kernel(
    A_x: jax.Array,
    A_wq: jax.Array,
    A_wk: jax.Array,
    A_wv: jax.Array,
    A_wo: jax.Array,
    B_x: jax.Array,
    B_w1: jax.Array,
    B_w2: jax.Array,
):
    del B_x
    out = pl.pallas_call(
        _KERNEL,
        out_shape=jax.ShapeDtypeStruct((D, S), bf16),
        in_specs=[pl.BlockSpec(memory_space=pl.ANY)] * 7,
        out_specs=pl.BlockSpec(memory_space=pl.ANY),
        scratch_shapes=_SCRATCH,
        compiler_params=pltpu.CompilerParams(vmem_limit_bytes=100 * 1024 * 1024),
    )(A_x.reshape(S, D).T, A_wq, A_wk.T, A_wv.T, A_wo, B_w1, B_w2.T)
    return out.T.reshape(1, S, D)
```

```python
import functools, math
import jax, jax.numpy as jnp
from jax import lax
from jax.experimental import pallas as pl
from jax.experimental.pallas import tpu as pltpu

S, D, H, DH, HP, F = 2048, 448, 16, 28, 32, 1792
EPS = 1e-5
bf16, f32, u32 = jnp.bfloat16, jnp.float32, jnp.uint32
QSCALE = (DH ** -0.5) * math.log2(math.e)
NT = (((1,), (1,)), ((), ()))
SAFE_BOUND = 36.0

def _ln_t(x):
    mean = jnp.sum(x, axis=0, keepdims=True) * (1.0 / D)
    xc = x - mean
    var = jnp.sum(xc * xc, axis=0, keepdims=True) * (1.0 / D)
    return (xc * lax.rsqrt(var + EPS)).astype(bf16)

def _dot(a, b):
    return jnp.dot(a, b, preferred_element_type=f32)

def _dot_nt(a, b):
    return lax.dot_general(a, b, NT, preferred_element_type=f32)

def _sel(rows, cols, fn):
    r = lax.broadcasted_iota(jnp.int32, (rows, cols), 0)
    c = lax.broadcasted_iota(jnp.int32, (rows, cols), 1)
    return jnp.where(fn(r, c), 1.0, 0.0).astype(bf16)

def make_kernel(T=512, CK=128, CB=256, skip=(), NVK=0, KT=4, FA=0.7, force=None, UN=2, QB=False, TS=1, XP=True):
    NB = S // T
    NJ = NB * H
    SM = S - NVK
    NL = T // 128
    NG = NVK // (8 * KT) if NVK else 0
    NCH = NL * NG

    def kernel(xt_hbm, wq_hbm, wkt_hbm, wvt_hbm, wo_hbm, w1_hbm, w2t_hbm, o_hbm,
               xin_ref, wq_ref, wkt_ref, wvt_ref, wo_ref, w1_ref, w2t_ref, xout_ref,
               xt_ref, qt_ref, ot_ref, k_ref, vt_ref, s_ref, p0_ref, p1_ref, ht_ref,
               wqt_ref, wkvt_ref, wot_ref, w1t_ref, kb_ref, qf_ref, qb_ref, nrm_ref, false_ref, sem_in, sem_w, sem_out):
        x_cp = [pltpu.make_async_copy(xt_hbm.at[:, b * T:(b + 1) * T], xin_ref.at[b], sem_in.at[b]) for b in range(NB)]
        w_cp = [pltpu.make_async_copy(src, dst, sem_w.at[i]) for i, (src, dst) in enumerate(
            [(wq_hbm, wq_ref), (wkt_hbm, wkt_ref), (wvt_hbm, wvt_ref), (wo_hbm, wo_ref), (w1_hbm, w1_ref), (w2t_hbm, w2t_ref)])]
        false_ref[...] = jnp.zeros((8, 128), jnp.int32)
        w_cp[0].start(); x_cp[0].start(); w_cp[1].start(); w_cp[2].start()

        G = 4 * DH
        eye128 = _sel(128, 128, lambda r, c: r == c)
        w_cp[0].wait(); w_cp[1].wait(); w_cp[2].wait(); x_cp[0].wait()
        for b in range(1, NB):
            x_cp[b].start()
        for n0 in range(0, D, 128):
            n1 = min(n0 + 128, D)
            wqt_ref[n0:n1, :] = _dot_nt(eye128[0:n1 - n0, 0:n1 - n0], wq_ref[:, n0:n1]).astype(bf16)
        wqt_ref[D:D + 2 * HP, :] = jnp.zeros((2 * HP, D), bf16)
        wqt_ref[D:D + DH, :] = wkt_ref[...]
        wqt_ref[D + HP:D + HP + DH, :] = wvt_ref[...]

        def qkv(b, x):
            ln = _ln_t(x)
            r = _dot(wqt_ref[...], ln)
            q = (r[0:D] * QSCALE).astype(bf16).astype(f32)
            heads, qns = [], []
            zpad = jnp.zeros((HP - DH - 1, T), f32)
            for h in range(H):
                qh = q[h * DH:(h + 1) * DH]
                qn = jnp.sqrt(jnp.sum(qh * qh, axis=0, keepdims=True))
                qns.append(qn)
                qt_ref[b, h * HP:(h + 1) * HP, :] = jnp.concatenate([qh, qn, zpad], axis=0).astype(bf16)
            qmax = qns[0]
            for qn in qns[1:]:
                qmax = jnp.maximum(qmax, qn)
            kb16 = r[D:D + HP].astype(bf16).astype(f32)
            kn2 = jnp.sum(kb16 * kb16, axis=0, keepdims=True)
            nrm_ref[b, 0:1, :] = qmax
            nrm_ref[b, 1:2, :] = kn2
            k_ref[pl.ds(pl.multiple_of(b * (T // 2), T // 2), T // 2), :] = pltpu.bitcast(kb16.T.astype(bf16), u32)
            row = lax.broadcasted_iota(jnp.int32, (HP, T), 0)
            vt_ref[b] = jnp.where(row == DH, 1.0, r[D + HP:D + 2 * HP]).astype(bf16)

        for b in range(NB):
            if b == 1:
                for bb in range(1, NB):
                    x_cp[bb].wait()
                w_cp[3].start(); w_cp[4].start(); w_cp[5].start()
            x = xin_ref[b].astype(f32)
            xt_ref[b] = x
            qkv(b, x)

        def wait_post_weights():
            w_cp[3].wait(); w_cp[4].wait(); w_cp[5].wait()

        def prep_post_weights_mxu():
            for n0 in range(0, D, 128):
                n1 = min(n0 + 128, D)
                wt = _dot_nt(eye128[0:n1 - n0, 0:n1 - n0], wo_ref[:, n0:n1]).astype(bf16)
                for g in range(4):
                    lo = (g * G) // 128 * 128
                    hi = min(-(-((g + 1) * G) // 128) * 128, D)
                    e = _sel(hi - lo, 128, lambda r, c: ((c % HP) < DH) & (r + lo == g * G + (c // HP) * DH + (c % HP)))
                    wot_ref[n0:n1, g * 128:(g + 1) * 128] = _dot(wt[:, lo:hi], e).astype(bf16)
            for j in range(F // 128):
                w1t_ref[j * 128:(j + 1) * 128, :] = _dot_nt(eye128, w1_ref[:, j * 128:(j + 1) * 128]).astype(bf16)

        def prep_post_weights_xlu(tok):
            false = false_ref[...] != 0
            n = F // 128 + 4
            def gated(x, i):
                t = tok(i, n)
                if t is None:
                    return x
                top = jnp.where(false, t, x[0:8, 0:128])
                if x.shape[1] > 128:
                    top = jnp.concatenate([top, x[0:8, 128:]], axis=1)
                return jnp.concatenate([top, x[8:]], axis=0)
            zrow = jnp.zeros((HP - DH, D), f32)
            for g in range(4):
                rows = []
                for h in range(4 * g, 4 * g + 4):
                    rows += [wo_ref[h * DH:(h + 1) * DH, :].astype(f32), zrow]
                blk = gated(jnp.concatenate(rows, axis=0), g)
                wot_ref[:, g * 128:(g + 1) * 128] = blk.T.astype(bf16)
            for j in range(F // 128):
                blk = gated(w1_ref[:, j * 128:(j + 1) * 128].astype(f32), 4 + j)
                w1t_ref[j * 128:(j + 1) * 128, :] = blk.T.astype(bf16)

        def load_q(j):
            return qt_ref[j // H, pl.ds(pl.multiple_of((j % H) * HP, HP), HP), :]

        def stage_c(jc, pc_ref, hook=None):
            acc = jnp.zeros((HP, T), f32)
            for c0 in range(0, S, CK):
                p = pltpu.bitcast(pc_ref[c0 // 2:(c0 + CK) // 2, :], bf16)
                kb, off = c0 // T, c0 % T
                part = _dot(vt_ref[kb, :, off:off + CK], p)
                if hook is not None:
                    hook(c0, part)
                acc = acc + part
            o = acc * (1.0 / acc[DH:DH + 1, :])
            ot_ref[jc // H, pl.ds(pl.multiple_of((jc % H) * HP, HP), HP), :] = o.astype(bf16)

        def step_safe(ja, jb_p_ref, mb, jc, pc_ref):
            if jb_p_ref is not None:
                for c0 in range(0, S, CB):
                    p = jnp.exp2(s_ref[c0:c0 + CB, :] - mb).astype(bf16)
                    jb_p_ref[c0 // 2:(c0 + CB) // 2, :] = pltpu.bitcast(p, u32)
            m = None
            if ja is not None:
                q = load_q(ja)
                row = lax.broadcasted_iota(jnp.int32, (HP, T), 0)
                q = jnp.where(row == DH, jnp.zeros_like(q), q)
                s = _dot(pltpu.bitcast(k_ref[...], bf16), q)
                s_ref[...] = s
                m = jnp.max(s, axis=0, keepdims=True)
            if jc is not None:
                stage_c(jc, pc_ref)
            return m

        def attention_safe(extra):
            if extra is not None:
                extra(lambda i, n: None)
            def body(j, c):
                m = step_safe(j, None, None, None, None)
                step_safe(None, p1_ref, m, None, None)
                @pl.when(j < NJ - 1)
                def _():
                    stage_c(j, p1_ref)
                return c
            lax.fori_loop(0, NJ, body, 0)

        def step_fast(ja, pa_ref, jc, pc_ref, vpu=True, extra=None):
            chains = []
            if ja is not None:
                q = load_q(ja)
                sm = SM if vpu else S
                s = _dot(pltpu.bitcast(k_ref[0:sm // 2, :], bf16), q)
                pa_ref[0:sm // 2, :] = pltpu.bitcast(jnp.exp2(s).astype(bf16), u32)
                if extra is not None:
                    extra(lambda i, n: s[((i * (sm // 8)) // n) * 8:((i * (sm // 8)) // n) * 8 + 8, 0:128])
                if NVK and vpu:
                    qf = q.astype(f32)
                    row = lax.broadcasted_iota(jnp.int32, (HP, T), 0)
                    qf = jnp.where(row == DH, qf * kb_ref[DH, 0:1, 0:1], qf)
                    if QB:
                        for d in range(DH + 1):
                            qb_ref[d] = jnp.broadcast_to(qf[d:d + 1, :], (8, T))
                    else:
                        qf_ref[...] = qf
                    false = false_ref[...] != 0

                    def chain(ci, tokens):
                        l, g = ci // NG, ci % NG
                        acc = None
                        for i, d in enumerate([DH] + list(range(DH))):
                            if QB:
                                qr = qb_ref[d, :, l * 128:(l + 1) * 128]
                            else:
                                qr = jnp.broadcast_to(qf_ref[d:d + 1, l * 128:(l + 1) * 128], (8, 128))
                            tok = tokens(i) if i % TS == 0 else None
                            if tok is not None:
                                qr = jnp.where(false, tok, qr)
                            qr = jnp.concatenate([qr] * KT, axis=0)
                            if d == DH:
                                acc = qr
                            else:
                                acc = acc + kb_ref[d, g * 8 * KT:(g + 1) * 8 * KT, :] * qr
                        r0 = SM + g * 8 * KT
                        pa_ref[r0 // 2:(r0 + 8 * KT) // 2, l * 128:(l + 1) * 128] = pltpu.bitcast(jnp.exp2(acc).astype(bf16), u32)

                    NA = NCH if jc is None else int(round(NCH * FA))
                    for ci in range(NA):
                        def tokens(i, ci=ci):
                            n = ci * (DH + 1) + i
                            r = (n * (SM // 8)) // (NA * (DH + 1))
                            l = ci // NG
                            return s[r * 8:(r + 1) * 8, l * 128:(l + 1) * 128]
                        chain(ci, tokens)
                    chains = list(range(NA, NCH))
            hook = None
            if chains:
                nsteps = len(chains) * (DH + 1)
                ntile = S // CK
                toks = {}
                def hook(c0, pu):
                    toks[c0 // CK] = pu
            if jc is not None:
                stage_c(jc, pc_ref, hook)
                for k, ci in enumerate(chains):
                    def tokens(i, k=k):
                        n = k * (DH + 1) + i
                        pos = (n * ntile * (HP // 8) * NL) // nsteps
                        t, rem = pos // ((HP // 8) * NL), pos % ((HP // 8) * NL)
                        r, l = rem // NL, rem % NL
                        return toks[t][r * 8:(r + 1) * 8, l * 128:(l + 1) * 128]
                    chain(ci, tokens)

        def attention_fast(kmax, extra):
            col = lax.broadcasted_iota(jnp.int32, (S // 2, HP), 1)
            nk = jnp.full((16, HP), -kmax, f32).astype(bf16)
            nk_u = pltpu.bitcast(nk, u32)[0:1, :]
            k_ref[...] = jnp.where(col == DH, nk_u, k_ref[...])
            if NVK:
                kf = pltpu.bitcast(k_ref[SM // 2:S // 2, :], bf16).astype(f32)
                for d in range(DH + 1):
                    kb_ref[d] = jnp.broadcast_to(kf[:, d:d + 1], (NVK, 128))
            step_fast(0, p0_ref, None, None, vpu=False, extra=extra)
            P = [p0_ref, p1_ref]
            NIT = (NJ - 2) // UN
            def body(jj, c):
                j = UN * jj
                for u in range(UN):
                    step_fast(j + u + 1, P[(u + 1) % 2], j + u, P[u % 2])
                return c
            lax.fori_loop(0, NIT, body, 0)
            for j in range(NIT * UN, NJ - 1):
                step_fast(j + 1, P[(j + 1) % 2], j, P[j % 2])

        def attention(extra=None):
            nr = nrm_ref[...]
            qmax = jnp.max(nr[:, 0:1, :])
            kmax = jnp.sqrt(jnp.max(nr[:, 1:2, :])) * 1.01
            safe = qmax * kmax <= SAFE_BOUND
            if force == 'fast':
                attention_fast(kmax, extra)
            elif force == 'safe':
                attention_safe(extra)
            else:
                @pl.when(safe)
                def _():
                    attention_fast(kmax, extra)
                @pl.when(jnp.logical_not(safe))
                def _():
                    attention_safe(extra)
            stage_c(NJ - 1, p1_ref)

        def out_cp(b):
            return pltpu.make_async_copy(xout_ref.at[b], o_hbm.at[:, pl.ds(pl.multiple_of(b * T, T), T)], sem_out.at[b])

        def post(layer):
            def body(b, carry):
                x = xt_ref[b] + _dot(wot_ref[...], ot_ref[b])
                ln = _ln_t(x)
                ht_ref[...] = jnp.maximum(_dot(w1t_ref[...], ln), 0.0).astype(bf16)
                x = x + _dot(w2t_ref[...], ht_ref[...])
                if layer == 0:
                    xt_ref[b] = x
                    qkv(b, x)
                else:
                    xout_ref[b] = x.astype(bf16)
                    out_cp(b).start()
                return carry
            lax.fori_loop(0, NB, body, 0)

        wait_post_weights()
        if 'attn' not in skip and XP:
            attention(prep_post_weights_xlu)
        else:
            if 'attn' not in skip: attention()
            prep_post_weights_mxu()
        if 'post' not in skip: post(0)
        if 'attn' not in skip: attention()
        post(1)
        for b in range(NB):
            out_cp(b).wait()

    scratch = [
        pltpu.VMEM((NB, D, T), bf16),
        pltpu.VMEM((D, D), bf16),
        pltpu.VMEM((DH, D), bf16),
        pltpu.VMEM((DH, D), bf16),
        pltpu.VMEM((D, D), bf16),
        pltpu.VMEM((D, F), bf16),
        pltpu.VMEM((D, F), bf16),
        pltpu.VMEM((NB, D, T), bf16),
        pltpu.VMEM((NB, D, T), f32),
        pltpu.VMEM((NB, H * HP, T), bf16),
        pltpu.VMEM((NB, H * HP, T), bf16),
        pltpu.VMEM((S // 2, HP), u32),
        pltpu.VMEM((NB, HP, T), bf16),
        pltpu.VMEM((S, T), f32),
        pltpu.VMEM((S // 2, T), u32),
        pltpu.VMEM((S // 2, T), u32),
        pltpu.VMEM((F, T), bf16),
        pltpu.VMEM((D + 2 * HP, D), bf16),
        pltpu.VMEM((2 * HP, D), bf16),
        pltpu.VMEM((D, H * HP), bf16),
        pltpu.VMEM((F, D), bf16),
        pltpu.VMEM((DH + 1, max(NVK, 8), 128), f32),
        pltpu.VMEM((HP, T), f32),
        pltpu.VMEM((DH + 1, 8, T), f32),
        pltpu.VMEM((NB, 2, T), f32),
        pltpu.VMEM((8, 128), jnp.int32),
        pltpu.SemaphoreType.DMA((NB,)),
        pltpu.SemaphoreType.DMA((6,)),
        pltpu.SemaphoreType.DMA((NB,)),
    ]
    return kernel, scratch


_KERNEL, _SCRATCH = make_kernel(NVK=224, FA=0.82, KT=7, QB=True, TS=2, UN=6)


@jax.jit
def pallas_interleave_layers__grouped_kv_mqa__dense_activation_relu__prompt_kernel(
    A_x: jax.Array,
    A_wq: jax.Array,
    A_wk: jax.Array,
    A_wv: jax.Array,
    A_wo: jax.Array,
    B_x: jax.Array,
    B_w1: jax.Array,
    B_w2: jax.Array,
):
    del B_x
    out = pl.pallas_call(
        _KERNEL,
        out_shape=jax.ShapeDtypeStruct((D, S), bf16),
        in_specs=[pl.BlockSpec(memory_space=pl.ANY)] * 7,
        out_specs=pl.BlockSpec(memory_space=pl.ANY),
        scratch_shapes=_SCRATCH,
        compiler_params=pltpu.CompilerParams(vmem_limit_bytes=100 * 1024 * 1024),
    )(A_x.reshape(S, D).T, A_wq, A_wk.T, A_wv.T, A_wo, B_w1, B_w2.T)
    return out.T.reshape(1, S, D)
```

```python
import math

import jax
import jax.numpy as jnp
from jax import lax
from jax.experimental import pallas as pl
from jax.experimental.pallas import tpu as pltpu

S, D, H, DH, F = 2048, 448, 16, 28, 1792
HP = 32
EPS = 1e-5
bf16, f32, u32 = jnp.bfloat16, jnp.float32, jnp.uint32
QSCALE = (DH ** -0.5) * math.log2(math.e)
SAFE_BOUND = 36.0

T = 512
NB = S // T
NJ = NB * H
NL = T // 128
CK = 128
CB = 256


def _ln_t(x):
    mean = jnp.sum(x, axis=0, keepdims=True) * (1.0 / D)
    xc = x - mean
    var = jnp.sum(xc * xc, axis=0, keepdims=True) * (1.0 / D)
    return (xc * lax.rsqrt(var + EPS)).astype(bf16)


def _dot(a, b):
    return jnp.dot(a, b, preferred_element_type=f32)


def _dot_nt(a, b):
    return lax.dot_general(a, b, (((1,), (1,)), ((), ())), preferred_element_type=f32)


def make_kernel(NVK=224, KT=7, FA=0.82, UN=6, TS=2, force=None):
    SM = S - NVK
    NG = NVK // (8 * KT)
    NCH = NL * NG

    def kernel(xt_hbm, wq_hbm, wkt_hbm, wvt_hbm, wo_hbm, w1_hbm, w2t_hbm, o_hbm,
               xin_ref, wq_ref, wkt_ref, wvt_ref, wo_ref, w1_ref, w2t_ref, xout_ref,
               xt_ref, qt_ref, ot_ref, k_ref, vt_ref, s_ref, p0_ref, p1_ref, ht_ref,
               wqt_ref, wot_ref, w1t_ref, kb_ref, qb_ref, nrm_ref, false_ref, sem_in, sem_w, sem_out):
        x_cp = [pltpu.make_async_copy(xt_hbm.at[:, b * T:(b + 1) * T], xin_ref.at[b], sem_in.at[b])
                for b in range(NB)]
        w_cp = [pltpu.make_async_copy(src, dst, sem_w.at[i]) for i, (src, dst) in enumerate(
            [(wq_hbm, wq_ref), (wkt_hbm, wkt_ref), (wvt_hbm, wvt_ref),
             (wo_hbm, wo_ref), (w1_hbm, w1_ref), (w2t_hbm, w2t_ref)])]
        false_ref[...] = jnp.zeros((8, 128), jnp.int32)
        w_cp[0].start(); x_cp[0].start(); w_cp[1].start(); w_cp[2].start()

        r_i = lax.broadcasted_iota(jnp.int32, (128, 128), 0)
        c_i = lax.broadcasted_iota(jnp.int32, (128, 128), 1)
        eye128 = jnp.where(r_i == c_i, 1.0, 0.0).astype(bf16)
        w_cp[0].wait(); w_cp[1].wait(); w_cp[2].wait(); x_cp[0].wait()
        for b in range(1, NB):
            x_cp[b].start()
        for n0 in range(0, D, 128):
            n1 = min(n0 + 128, D)
            wqt_ref[n0:n1, :] = _dot_nt(eye128[0:n1 - n0, 0:n1 - n0], wq_ref[:, n0:n1]).astype(bf16)
        wqt_ref[D:D + 2 * HP, :] = jnp.zeros((2 * HP, D), bf16)
        wqt_ref[D:D + DH, :] = wkt_ref[...]
        wqt_ref[D + HP:D + HP + DH, :] = wvt_ref[...]

        def qkv_mm(x):
            return _dot(wqt_ref[...], _ln_t(x))

        def qkv_post(b, r):
            q = (r[0:D] * QSCALE).astype(bf16).astype(f32)
            qns = []
            zpad = jnp.zeros((HP - DH - 1, T), f32)
            for h in range(H):
                qh = q[h * DH:(h + 1) * DH]
                qn = jnp.sqrt(jnp.sum(qh * qh, axis=0, keepdims=True))
                qns.append(qn)
                qt_ref[b, h * HP:(h + 1) * HP, :] = jnp.concatenate([qh, qn, zpad], axis=0).astype(bf16)
            qmax = qns[0]
            for qn in qns[1:]:
                qmax = jnp.maximum(qmax, qn)
            kb16 = r[D:D + HP].astype(bf16).astype(f32)
            kn2 = jnp.sum(kb16 * kb16, axis=0, keepdims=True)
            nrm_ref[b, 0:1, :] = qmax
            nrm_ref[b, 1:2, :] = kn2
            row = lax.broadcasted_iota(jnp.int32, (HP, T), 0)
            kb16 = jnp.where(row == DH, 1.0, kb16)
            k_ref[pl.ds(pl.multiple_of(b * (T // 2), T // 2), T // 2), :] = pltpu.bitcast(kb16.T.astype(bf16), u32)
            vt_ref[b] = jnp.where(row == DH, 1.0, r[D + HP:D + 2 * HP]).astype(bf16)

        for b in range(NB):
            x = xin_ref[b].astype(f32)
            xt_ref[b] = x
            r = qkv_mm(x)
            if b == 0:
                for bb in range(1, NB):
                    x_cp[bb].wait()
                w_cp[3].start(); w_cp[4].start(); w_cp[5].start()
            qkv_post(b, r)

        def prep_post_weights(tok):
            false = false_ref[...] != 0
            n = F // 128 + 4

            def gated(x, i):
                t = tok(i, n)
                if t is None:
                    return x
                top = jnp.where(false, t, x[0:8, 0:128])
                if x.shape[1] > 128:
                    top = jnp.concatenate([top, x[0:8, 128:]], axis=1)
                return jnp.concatenate([top, x[8:]], axis=0)

            zrow = jnp.zeros((HP - DH, D), f32)
            for g in range(4):
                rows = []
                for h in range(4 * g, 4 * g + 4):
                    rows += [wo_ref[h * DH:(h + 1) * DH, :].astype(f32), zrow]
                blk = gated(jnp.concatenate(rows, axis=0), g)
                wot_ref[:, g * 128:(g + 1) * 128] = blk.T.astype(bf16)
            for j in range(F // 128):
                blk = gated(w1_ref[:, j * 128:(j + 1) * 128].astype(f32), 4 + j)
                w1t_ref[j * 128:(j + 1) * 128, :] = blk.T.astype(bf16)

        def load_q(j):
            return qt_ref[j // H, pl.ds(pl.multiple_of((j % H) * HP, HP), HP), :]

        def stage_pv(j, p_ref, hook=None):
            acc = jnp.zeros((HP, T), f32)
            for c0 in range(0, S, CK):
                p = pltpu.bitcast(p_ref[c0 // 2:(c0 + CK) // 2, :], bf16)
                part = _dot(vt_ref[c0 // T, :, c0 % T:c0 % T + CK], p)
                if hook is not None:
                    hook(c0, part)
                acc = acc + part
            o = acc * (1.0 / acc[DH:DH + 1, :])
            ot_ref[j // H, pl.ds(pl.multiple_of((j % H) * HP, HP), HP), :] = o.astype(bf16)

        def attention_exact(extra):
            if extra is not None:
                extra(lambda i, n: None)

            def body(j, c):
                q = load_q(j)
                row = lax.broadcasted_iota(jnp.int32, (HP, T), 0)
                q = jnp.where(row == DH, jnp.zeros_like(q), q)
                s = _dot(pltpu.bitcast(k_ref[...], bf16), q)
                s_ref[...] = s
                m = jnp.max(s, axis=0, keepdims=True)
                for c0 in range(0, S, CB):
                    p = jnp.exp2(s_ref[c0:c0 + CB, :] - m).astype(bf16)
                    p1_ref[c0 // 2:(c0 + CB) // 2, :] = pltpu.bitcast(p, u32)

                @pl.when(j < NJ - 1)
                def _():
                    stage_pv(j, p1_ref)
                return c
            lax.fori_loop(0, NJ, body, 0)

        def step(nkmax, ja, pa_ref, jc, pc_ref, vpu=True, extra=None):
            row = lax.broadcasted_iota(jnp.int32, (HP, T), 0)
            qf = load_q(ja).astype(f32)
            q = jnp.where(row == DH, qf * nkmax, qf).astype(bf16)
            sm = SM if vpu else S
            s = _dot(pltpu.bitcast(k_ref[0:sm // 2, :], bf16), q)
            pa_ref[0:sm // 2, :] = pltpu.bitcast(jnp.exp2(s).astype(bf16), u32)
            if extra is not None:
                extra(lambda i, n: s[((i * (sm // 8)) // n) * 8:((i * (sm // 8)) // n) * 8 + 8, 0:128])
            late = []
            if vpu:
                qf = q.astype(f32)
                for d in range(DH + 1):
                    qb_ref[d] = jnp.broadcast_to(qf[d:d + 1, :], (8, T))
                false = false_ref[...] != 0

                def chain(ci, tokens):
                    l, g = ci // NG, ci % NG
                    acc = None
                    for i, d in enumerate([DH] + list(range(DH))):
                        qr = qb_ref[d, :, l * 128:(l + 1) * 128]
                        if i % TS == 0:
                            qr = jnp.where(false, tokens(i), qr)
                        qr = jnp.concatenate([qr] * KT, axis=0)
                        if d == DH:
                            acc = qr
                        else:
                            acc = acc + kb_ref[d, g * 8 * KT:(g + 1) * 8 * KT, :] * qr
                    r0 = SM + g * 8 * KT
                    pa_ref[r0 // 2:(r0 + 8 * KT) // 2, l * 128:(l + 1) * 128] = pltpu.bitcast(
                        jnp.exp2(acc).astype(bf16), u32)

                na = int(round(NCH * FA))
                for ci in range(na):
                    def tokens(i, ci=ci):
                        n = ci * (DH + 1) + i
                        r = (n * (SM // 8)) // (na * (DH + 1))
                        l = ci // NG
                        return s[r * 8:(r + 1) * 8, l * 128:(l + 1) * 128]
                    chain(ci, tokens)
                late = list(range(na, NCH))
            if jc is not None:
                parts = {}
                stage_pv(jc, pc_ref, lambda c0, part: parts.__setitem__(c0 // CK, part))
                nsteps = len(late) * (DH + 1)
                per = (HP // 8) * NL
                for k, ci in enumerate(late):
                    def tokens(i, k=k):
                        pos = ((k * (DH + 1) + i) * (S // CK) * per) // nsteps
                        t, rem = pos // per, pos % per
                        r, l = rem // NL, rem % NL
                        return parts[t][r * 8:(r + 1) * 8, l * 128:(l + 1) * 128]
                    chain(ci, tokens)

        def attention_bounded(kmax, extra):
            nkmax = -kmax
            kf = pltpu.bitcast(k_ref[SM // 2:S // 2, :], bf16).astype(f32)
            for d in range(DH):
                kb_ref[d] = jnp.broadcast_to(kf[:, d:d + 1], (NVK, 128))
            step(nkmax, 0, p0_ref, None, None, vpu=False, extra=extra)
            P = [p0_ref, p1_ref]
            nit = (NJ - 2) // UN

            def body(jj, c):
                j = UN * jj
                for u in range(UN):
                    step(nkmax, j + u + 1, P[(u + 1) % 2], j + u, P[u % 2])
                return c
            lax.fori_loop(0, nit, body, 0)
            for j in range(nit * UN, NJ - 1):
                step(nkmax, j + 1, P[(j + 1) % 2], j, P[j % 2])

        def attention(extra=None):
            nr = nrm_ref[...]
            qmax = jnp.max(nr[:, 0:1, :])
            kmax = jnp.sqrt(jnp.max(nr[:, 1:2, :])) * 1.01
            safe = qmax * kmax <= SAFE_BOUND
            if force == 'fast':
                attention_bounded(kmax, extra)
            elif force == 'safe':
                attention_exact(extra)
            else:
                @pl.when(safe)
                def _():
                    attention_bounded(kmax, extra)

                @pl.when(jnp.logical_not(safe))
                def _():
                    attention_exact(extra)
            stage_pv(NJ - 1, p1_ref)

        def out_cp(b):
            return pltpu.make_async_copy(xout_ref.at[b], o_hbm.at[:, pl.ds(pl.multiple_of(b * T, T), T)],
                                         sem_out.at[b])

        def post(layer):
            def body(b, carry):
                x = xt_ref[b] + _dot(wot_ref[...], ot_ref[b])
                ln = _ln_t(x)
                ht_ref[...] = jnp.maximum(_dot(w1t_ref[...], ln), 0.0).astype(bf16)
                x = x + _dot(w2t_ref[...], ht_ref[...])
                if layer == 0:
                    xt_ref[b] = x
                    qkv_post(b, qkv_mm(x))
                else:
                    xout_ref[b] = x.astype(bf16)
                    out_cp(b).start()
                return carry
            lax.fori_loop(0, NB, body, 0)

        w_cp[3].wait(); w_cp[4].wait(); w_cp[5].wait()
        attention(prep_post_weights)
        post(0)
        attention()
        post(1)
        for b in range(NB):
            out_cp(b).wait()

    scratch = [
        pltpu.VMEM((NB, D, T), bf16),
        pltpu.VMEM((D, D), bf16),
        pltpu.VMEM((DH, D), bf16),
        pltpu.VMEM((DH, D), bf16),
        pltpu.VMEM((D, D), bf16),
        pltpu.VMEM((D, F), bf16),
        pltpu.VMEM((D, F), bf16),
        pltpu.VMEM((NB, D, T), bf16),
        pltpu.VMEM((NB, D, T), f32),
        pltpu.VMEM((NB, H * HP, T), bf16),
        pltpu.VMEM((NB, H * HP, T), bf16),
        pltpu.VMEM((S // 2, HP), u32),
        pltpu.VMEM((NB, HP, T), bf16),
        pltpu.VMEM((S, T), f32),
        pltpu.VMEM((S // 2, T), u32),
        pltpu.VMEM((S // 2, T), u32),
        pltpu.VMEM((F, T), bf16),
        pltpu.VMEM((D + 2 * HP, D), bf16),
        pltpu.VMEM((D, H * HP), bf16),
        pltpu.VMEM((F, D), bf16),
        pltpu.VMEM((DH, NVK, 128), f32),
        pltpu.VMEM((DH + 1, 8, T), f32),
        pltpu.VMEM((NB, 2, T), f32),
        pltpu.VMEM((8, 128), jnp.int32),
        pltpu.SemaphoreType.DMA((NB,)),
        pltpu.SemaphoreType.DMA((6,)),
        pltpu.SemaphoreType.DMA((NB,)),
    ]
    return kernel, scratch


_KERNEL, _SCRATCH = make_kernel()


@jax.jit
def pallas_interleave_layers__grouped_kv_mqa__dense_activation_relu__prompt_kernel(
    A_x: jax.Array,
    A_wq: jax.Array,
    A_wk: jax.Array,
    A_wv: jax.Array,
    A_wo: jax.Array,
    B_x: jax.Array,
    B_w1: jax.Array,
    B_w2: jax.Array,
):
    del B_x
    out = pl.pallas_call(
        _KERNEL,
        out_shape=jax.ShapeDtypeStruct((D, S), bf16),
        in_specs=[pl.BlockSpec(memory_space=pl.ANY)] * 7,
        out_specs=pl.BlockSpec(memory_space=pl.ANY),
        scratch_shapes=_SCRATCH,
        compiler_params=pltpu.CompilerParams(vmem_limit_bytes=100 * 1024 * 1024),
    )(A_x.reshape(S, D).T, A_wq, A_wk.T, A_wv.T, A_wo, B_w1, B_w2.T)
    return out.T.reshape(1, S, D)
```

```python
import math

import jax
import jax.numpy as jnp
from jax import lax
from jax.experimental import pallas as pl
from jax.experimental.pallas import tpu as pltpu

S, D, H, DH, F = 2048, 448, 16, 28, 1792
HP = 32
EPS = 1e-5
bf16, f32, u32 = jnp.bfloat16, jnp.float32, jnp.uint32
QSCALE = (DH ** -0.5) * math.log2(math.e)
SAFE_BOUND = 36.0

T = 512
NB = S // T
NJ = NB * H
NL = T // 128
CK = 128
CB = 256


def _ln_t(x):
    mean = jnp.sum(x, axis=0, keepdims=True) * (1.0 / D)
    xc = x - mean
    var = jnp.sum(xc * xc, axis=0, keepdims=True) * (1.0 / D)
    return (xc * lax.rsqrt(var + EPS)).astype(bf16)


def _dot(a, b):
    return jnp.dot(a, b, preferred_element_type=f32)


def _dot_nt(a, b):
    return lax.dot_general(a, b, (((1,), (1,)), ((), ())), preferred_element_type=f32)


def make_kernel(NVK=240, KT=6, FA=0.8, UN=9, TS=2, NP=3, force=None):
    SM = S - NVK
    NG = NVK // (8 * KT)
    NCH = NL * NG

    def kernel(xt_hbm, wq_hbm, wkt_hbm, wvt_hbm, wo_hbm, w1_hbm, w2t_hbm, o_hbm,
               xin_ref, wq_ref, wkt_ref, wvt_ref, wo_ref, w1_ref, w2t_ref, xout_ref,
               xt_ref, qt_ref, ot_ref, k_ref, vt_ref, s_ref, p0_ref, p1_ref, p2_ref, ht_ref,
               wqt_ref, wot_ref, w1t_ref, kb_ref, qb_ref, nrm_ref, false_ref, sem_in, sem_w, sem_out):
        P = [p0_ref, p1_ref, p2_ref][:NP]
        plast_ref = P[(NJ - 1) % NP]
        x_cp = [pltpu.make_async_copy(xt_hbm.at[:, b * T:(b + 1) * T], xin_ref.at[b], sem_in.at[b])
                for b in range(NB)]
        w_cp = [pltpu.make_async_copy(src, dst, sem_w.at[i]) for i, (src, dst) in enumerate(
            [(wq_hbm, wq_ref), (wkt_hbm, wkt_ref), (wvt_hbm, wvt_ref),
             (wo_hbm, wo_ref), (w1_hbm, w1_ref), (w2t_hbm, w2t_ref)])]
        false_ref[...] = jnp.zeros((8, 128), jnp.int32)
        w_cp[0].start(); x_cp[0].start(); w_cp[1].start(); w_cp[2].start()

        r_i = lax.broadcasted_iota(jnp.int32, (128, 128), 0)
        c_i = lax.broadcasted_iota(jnp.int32, (128, 128), 1)
        eye128 = jnp.where(r_i == c_i, 1.0, 0.0).astype(bf16)
        w_cp[0].wait(); w_cp[1].wait(); w_cp[2].wait(); x_cp[0].wait()
        for b in range(1, NB):
            x_cp[b].start()
        for n0 in range(0, D, 128):
            n1 = min(n0 + 128, D)
            wqt_ref[n0:n1, :] = _dot_nt(eye128[0:n1 - n0, 0:n1 - n0], wq_ref[:, n0:n1]).astype(bf16)
        wqt_ref[D:D + 2 * HP, :] = jnp.zeros((2 * HP, D), bf16)
        wqt_ref[D:D + DH, :] = wkt_ref[...]
        wqt_ref[D + HP:D + HP + DH, :] = wvt_ref[...]

        def qkv_mm(x):
            return _dot(wqt_ref[...], _ln_t(x))

        def qkv_post(b, r):
            q = (r[0:D] * QSCALE).astype(bf16).astype(f32)
            qns = []
            zpad = jnp.zeros((HP - DH - 1, T), f32)
            for h in range(H):
                qh = q[h * DH:(h + 1) * DH]
                qn = jnp.sqrt(jnp.sum(qh * qh, axis=0, keepdims=True))
                qns.append(qn)
                qt_ref[b, h * HP:(h + 1) * HP, :] = jnp.concatenate([qh, qn, zpad], axis=0).astype(bf16)
            qmax = qns[0]
            for qn in qns[1:]:
                qmax = jnp.maximum(qmax, qn)
            kb16 = r[D:D + HP].astype(bf16).astype(f32)
            kn2 = jnp.sum(kb16 * kb16, axis=0, keepdims=True)
            nrm_ref[b, 0:1, :] = qmax
            nrm_ref[b, 1:2, :] = kn2
            row = lax.broadcasted_iota(jnp.int32, (HP, T), 0)
            kb16 = jnp.where(row == DH, 1.0, kb16)
            k_ref[pl.ds(pl.multiple_of(b * (T // 2), T // 2), T // 2), :] = pltpu.bitcast(kb16.T.astype(bf16), u32)
            vt_ref[b] = jnp.where(row == DH, 1.0, r[D + HP:D + 2 * HP]).astype(bf16)

        for b in range(NB):
            x = xin_ref[b].astype(f32)
            xt_ref[b] = x
            r = qkv_mm(x)
            if b == 0:
                for bb in range(1, NB):
                    x_cp[bb].wait()
                w_cp[3].start(); w_cp[4].start(); w_cp[5].start()
            qkv_post(b, r)

        def prep_post_weights(tok):
            false = false_ref[...] != 0
            n = F // 128 + 4

            def gated(x, i):
                t = tok(i, n)
                if t is None:
                    return x
                top = jnp.where(false, t, x[0:8, 0:128])
                if x.shape[1] > 128:
                    top = jnp.concatenate([top, x[0:8, 128:]], axis=1)
                return jnp.concatenate([top, x[8:]], axis=0)

            zrow = jnp.zeros((HP - DH, D), f32)
            for g in range(4):
                rows = []
                for h in range(4 * g, 4 * g + 4):
                    rows += [wo_ref[h * DH:(h + 1) * DH, :].astype(f32), zrow]
                blk = gated(jnp.concatenate(rows, axis=0), g)
                wot_ref[:, g * 128:(g + 1) * 128] = blk.T.astype(bf16)
            for j in range(F // 128):
                blk = gated(w1_ref[:, j * 128:(j + 1) * 128].astype(f32), 4 + j)
                w1t_ref[j * 128:(j + 1) * 128, :] = blk.T.astype(bf16)

        def load_q(j):
            return qt_ref[j // H, pl.ds(pl.multiple_of((j % H) * HP, HP), HP), :]

        def stage_pv(j, p_ref, hook=None):
            acc = jnp.zeros((HP, T), f32)
            for c0 in range(0, S, CK):
                p = pltpu.bitcast(p_ref[c0 // 2:(c0 + CK) // 2, :], bf16)
                part = _dot(vt_ref[c0 // T, :, c0 % T:c0 % T + CK], p)
                if hook is not None:
                    hook(c0, part)
                acc = acc + part
            o = acc * (1.0 / acc[DH:DH + 1, :])
            ot_ref[j // H, pl.ds(pl.multiple_of((j % H) * HP, HP), HP), :] = o.astype(bf16)

        def attention_exact(extra):
            if extra is not None:
                extra(lambda i, n: None)

            def body(j, c):
                q = load_q(j)
                row = lax.broadcasted_iota(jnp.int32, (HP, T), 0)
                q = jnp.where(row == DH, jnp.zeros_like(q), q)
                s = _dot(pltpu.bitcast(k_ref[...], bf16), q)
                s_ref[...] = s
                m = jnp.max(s, axis=0, keepdims=True)
                for c0 in range(0, S, CB):
                    p = jnp.exp2(s_ref[c0:c0 + CB, :] - m).astype(bf16)
                    plast_ref[c0 // 2:(c0 + CB) // 2, :] = pltpu.bitcast(p, u32)

                @pl.when(j < NJ - 1)
                def _():
                    stage_pv(j, plast_ref)
                return c
            lax.fori_loop(0, NJ, body, 0)

        def step(nkmax, ja, pa_ref, jc, pc_ref, vpu=True, extra=None):
            row = lax.broadcasted_iota(jnp.int32, (HP, T), 0)
            qf = load_q(ja).astype(f32)
            q = jnp.where(row == DH, qf * nkmax, qf).astype(bf16)
            sm = SM if vpu else S
            s = _dot(pltpu.bitcast(k_ref[0:sm // 2, :], bf16), q)
            pa_ref[0:sm // 2, :] = pltpu.bitcast(jnp.exp2(s).astype(bf16), u32)
            if extra is not None:
                extra(lambda i, n: s[((i * (sm // 8)) // n) * 8:((i * (sm // 8)) // n) * 8 + 8, 0:128])
            late = []
            if vpu:
                qf = q.astype(f32)
                for d in range(DH + 1):
                    qb_ref[d] = jnp.broadcast_to(qf[d:d + 1, :], (8, T))
                false = false_ref[...] != 0

                def chain(ci, tokens):
                    l, g = ci // NG, ci % NG
                    acc = None
                    for i, d in enumerate([DH] + list(range(DH))):
                        qr = qb_ref[d, :, l * 128:(l + 1) * 128]
                        if i % TS == 0:
                            qr = jnp.where(false, tokens(i), qr)
                        qr = jnp.concatenate([qr] * KT, axis=0)
                        if d == DH:
                            acc = qr
                        else:
                            acc = acc + kb_ref[d, g * 8 * KT:(g + 1) * 8 * KT, :] * qr
                    r0 = SM + g * 8 * KT
                    pa_ref[r0 // 2:(r0 + 8 * KT) // 2, l * 128:(l + 1) * 128] = pltpu.bitcast(
                        jnp.exp2(acc).astype(bf16), u32)

                na = int(round(NCH * FA))
                for ci in range(na):
                    def tokens(i, ci=ci):
                        n = ci * (DH + 1) + i
                        r = (n * (SM // 8)) // (na * (DH + 1))
                        l = ci // NG
                        return s[r * 8:(r + 1) * 8, l * 128:(l + 1) * 128]
                    chain(ci, tokens)
                late = list(range(na, NCH))
            if jc is not None:
                parts = {}
                stage_pv(jc, pc_ref, lambda c0, part: parts.__setitem__(c0 // CK, part))
                nsteps = len(late) * (DH + 1)
                per = (HP // 8) * NL
                for k, ci in enumerate(late):
                    def tokens(i, k=k):
                        pos = ((k * (DH + 1) + i) * (S // CK) * per) // nsteps
                        t, rem = pos // per, pos % per
                        r, l = rem // NL, rem % NL
                        return parts[t][r * 8:(r + 1) * 8, l * 128:(l + 1) * 128]
                    chain(ci, tokens)

        def attention_bounded(kmax, extra):
            nkmax = -kmax
            kf = pltpu.bitcast(k_ref[SM // 2:S // 2, :], bf16).astype(f32)
            for d in range(DH):
                kb_ref[d] = jnp.broadcast_to(kf[:, d:d + 1], (NVK, 128))
            step(nkmax, 0, p0_ref, None, None, vpu=False, extra=extra)
            assert UN % NP == 0
            nit = (NJ - 1) // UN

            def body(jj, c):
                j = UN * jj
                for u in range(UN):
                    step(nkmax, j + u + 1, P[(u + 1) % NP], j + u, P[u % NP])
                return c
            lax.fori_loop(0, nit, body, 0)
            for j in range(nit * UN, NJ - 1):
                step(nkmax, j + 1, P[(j + 1) % NP], j, P[j % NP])

        def attention(extra=None):
            nr = nrm_ref[...]
            qmax = jnp.max(nr[:, 0:1, :])
            kmax = jnp.sqrt(jnp.max(nr[:, 1:2, :])) * 1.01
            safe = qmax * kmax <= SAFE_BOUND
            if force == 'fast':
                attention_bounded(kmax, extra)
            elif force == 'safe':
                attention_exact(extra)
            else:
                @pl.when(safe)
                def _():
                    attention_bounded(kmax, extra)

                @pl.when(jnp.logical_not(safe))
                def _():
                    attention_exact(extra)
            stage_pv(NJ - 1, plast_ref)

        def out_cp(b):
            return pltpu.make_async_copy(xout_ref.at[b], o_hbm.at[:, pl.ds(pl.multiple_of(b * T, T), T)],
                                         sem_out.at[b])

        def post(layer):
            def body(b, carry):
                x = xt_ref[b] + _dot(wot_ref[...], ot_ref[b])
                ln = _ln_t(x)
                ht_ref[...] = jnp.maximum(_dot(w1t_ref[...], ln), 0.0).astype(bf16)
                x = x + _dot(w2t_ref[...], ht_ref[...])
                if layer == 0:
                    xt_ref[b] = x
                    qkv_post(b, qkv_mm(x))
                else:
                    xout_ref[b] = x.astype(bf16)
                    out_cp(b).start()
                return carry
            lax.fori_loop(0, NB, body, 0)

        w_cp[3].wait(); w_cp[4].wait(); w_cp[5].wait()
        attention(prep_post_weights)
        post(0)
        attention()
        post(1)
        for b in range(NB):
            out_cp(b).wait()

    scratch = [
        pltpu.VMEM((NB, D, T), bf16),
        pltpu.VMEM((D, D), bf16),
        pltpu.VMEM((DH, D), bf16),
        pltpu.VMEM((DH, D), bf16),
        pltpu.VMEM((D, D), bf16),
        pltpu.VMEM((D, F), bf16),
        pltpu.VMEM((D, F), bf16),
        pltpu.VMEM((NB, D, T), bf16),
        pltpu.VMEM((NB, D, T), f32),
        pltpu.VMEM((NB, H * HP, T), bf16),
        pltpu.VMEM((NB, H * HP, T), bf16),
        pltpu.VMEM((S // 2, HP), u32),
        pltpu.VMEM((NB, HP, T), bf16),
        pltpu.VMEM((S, T), f32),
        pltpu.VMEM((S // 2, T), u32),
        pltpu.VMEM((S // 2, T), u32),
        pltpu.VMEM((S // 2, T), u32),
        pltpu.VMEM((F, T), bf16),
        pltpu.VMEM((D + 2 * HP, D), bf16),
        pltpu.VMEM((D, H * HP), bf16),
        pltpu.VMEM((F, D), bf16),
        pltpu.VMEM((DH, NVK, 128), f32),
        pltpu.VMEM((DH + 1, 8, T), f32),
        pltpu.VMEM((NB, 2, T), f32),
        pltpu.VMEM((8, 128), jnp.int32),
        pltpu.SemaphoreType.DMA((NB,)),
        pltpu.SemaphoreType.DMA((6,)),
        pltpu.SemaphoreType.DMA((NB,)),
    ]
    return kernel, scratch


_KERNEL, _SCRATCH = make_kernel()


@jax.jit
def pallas_interleave_layers__grouped_kv_mqa__dense_activation_relu__prompt_kernel(
    A_x: jax.Array,
    A_wq: jax.Array,
    A_wk: jax.Array,
    A_wv: jax.Array,
    A_wo: jax.Array,
    B_x: jax.Array,
    B_w1: jax.Array,
    B_w2: jax.Array,
):
    del B_x
    out = pl.pallas_call(
        _KERNEL,
        out_shape=jax.ShapeDtypeStruct((D, S), bf16),
        in_specs=[pl.BlockSpec(memory_space=pl.ANY)] * 7,
        out_specs=pl.BlockSpec(memory_space=pl.ANY),
        scratch_shapes=_SCRATCH,
        compiler_params=pltpu.CompilerParams(vmem_limit_bytes=100 * 1024 * 1024),
    )(A_x.reshape(S, D).T, A_wq, A_wk.T, A_wv.T, A_wo, B_w1, B_w2.T)
    return out.T.reshape(1, S, D)
```

```python
import math

import jax
import jax.numpy as jnp
from jax import lax
from jax.experimental import pallas as pl
from jax.experimental.pallas import tpu as pltpu

S, D, H, DH, F = 2048, 448, 16, 28, 1792
HP = 32
EPS = 1e-5
bf16, f32, u32 = jnp.bfloat16, jnp.float32, jnp.uint32
QSCALE = (DH ** -0.5) * math.log2(math.e)
SAFE_BOUND = 36.0

T = 512
NB = S // T
NJ = NB * H
NL = T // 128
CK = 128
CB = 256


def _ln_t(x):
    mean = jnp.sum(x, axis=0, keepdims=True) * (1.0 / D)
    xc = x - mean
    var = jnp.sum(xc * xc, axis=0, keepdims=True) * (1.0 / D)
    return (xc * lax.rsqrt(var + EPS)).astype(bf16)


def _dot(a, b):
    return jnp.dot(a, b, preferred_element_type=f32)


def _dot_nt(a, b):
    return lax.dot_general(a, b, (((1,), (1,)), ((), ())), preferred_element_type=f32)


def make_kernel(NVK=240, KT=6, FA=0.8, UN=9, TS=2, NP=3, force=None):
    SM = S - NVK
    NG = NVK // (8 * KT)
    NCH = NL * NG

    def kernel(xt_hbm, wq_hbm, wkt_hbm, wvt_hbm, wo_hbm, w1_hbm, w2t_hbm, o_hbm,
               xin_ref, wq_ref, wkt_ref, wvt_ref, wo_ref, w1_ref, w2t_ref, xout_ref,
               xt_ref, qt_ref, ot_ref, k_ref, vt_ref, s_ref, p0_ref, p1_ref, p2_ref, ht_ref,
               wqt_ref, wot_ref, w1t_ref, kb_ref, qb_ref, nrm_ref, false_ref, sem_in, sem_w, sem_out):
        P = [p0_ref, p1_ref, p2_ref][:NP]
        plast_ref = P[(NJ - 1) % NP]
        x_cp = [pltpu.make_async_copy(xt_hbm.at[:, b * T:(b + 1) * T], xin_ref.at[b], sem_in.at[b])
                for b in range(NB)]
        w_cp = [pltpu.make_async_copy(src, dst, sem_w.at[i]) for i, (src, dst) in enumerate(
            [(wq_hbm, wq_ref), (wkt_hbm, wkt_ref), (wvt_hbm, wvt_ref),
             (wo_hbm, wo_ref), (w1_hbm, w1_ref), (w2t_hbm, w2t_ref)])]
        false_ref[...] = jnp.zeros((8, 128), jnp.int32)
        w_cp[0].start(); x_cp[0].start(); w_cp[1].start(); w_cp[2].start()

        r_i = lax.broadcasted_iota(jnp.int32, (128, 128), 0)
        c_i = lax.broadcasted_iota(jnp.int32, (128, 128), 1)
        eye128 = jnp.where(r_i == c_i, 1.0, 0.0).astype(bf16)
        w_cp[0].wait(); w_cp[1].wait(); w_cp[2].wait(); x_cp[0].wait()
        for b in range(1, NB):
            x_cp[b].start()
        for n0 in range(0, D, 128):
            n1 = min(n0 + 128, D)
            wqt_ref[n0:n1, :] = _dot_nt(eye128[0:n1 - n0, 0:n1 - n0], wq_ref[:, n0:n1]).astype(bf16)
        wqt_ref[D:D + 2 * HP, :] = jnp.zeros((2 * HP, D), bf16)
        wqt_ref[D:D + DH, :] = wkt_ref[...]
        wqt_ref[D + HP:D + HP + DH, :] = wvt_ref[...]

        def qkv_mm(x):
            return _dot(wqt_ref[...], _ln_t(x))

        def qkv_post(b, r):
            q = (r[0:D] * QSCALE).astype(bf16).astype(f32)
            qns = []
            zpad = jnp.zeros((HP - DH - 1, T), f32)
            for h in range(H):
                qh = q[h * DH:(h + 1) * DH]
                qn = jnp.sqrt(jnp.sum(qh * qh, axis=0, keepdims=True))
                qns.append(qn)
                qt_ref[b, h * HP:(h + 1) * HP, :] = jnp.concatenate([qh, qn, zpad], axis=0).astype(bf16)
            qmax = qns[0]
            for qn in qns[1:]:
                qmax = jnp.maximum(qmax, qn)
            kb16 = r[D:D + HP].astype(bf16).astype(f32)
            kn2 = jnp.sum(kb16 * kb16, axis=0, keepdims=True)
            nrm_ref[b, 0:1, :] = qmax
            nrm_ref[b, 1:2, :] = kn2
            row = lax.broadcasted_iota(jnp.int32, (HP, T), 0)
            kb16 = jnp.where(row == DH, 1.0, kb16)
            k_ref[pl.ds(pl.multiple_of(b * (T // 2), T // 2), T // 2), :] = pltpu.bitcast(kb16.T.astype(bf16), u32)
            vt_ref[b] = jnp.where(row == DH, 1.0, r[D + HP:D + 2 * HP]).astype(bf16)

        for b in range(NB):
            x = xin_ref[b].astype(f32)
            xt_ref[b] = x
            r = qkv_mm(x)
            if b == 0:
                for bb in range(1, NB):
                    x_cp[bb].wait()
                w_cp[3].start(); w_cp[4].start(); w_cp[5].start()
            qkv_post(b, r)

        def prep_post_weights(tok):
            false = false_ref[...] != 0
            n = F // 128 + 4

            def gated(x, i):
                t = tok(i, n)
                if t is None:
                    return x
                top = jnp.where(false, t, x[0:8, 0:128])
                if x.shape[1] > 128:
                    top = jnp.concatenate([top, x[0:8, 128:]], axis=1)
                return jnp.concatenate([top, x[8:]], axis=0)

            zrow = jnp.zeros((HP - DH, D), f32)
            for g in range(4):
                rows = []
                for h in range(4 * g, 4 * g + 4):
                    rows += [wo_ref[h * DH:(h + 1) * DH, :].astype(f32), zrow]
                blk = gated(jnp.concatenate(rows, axis=0), g)
                wot_ref[:, g * 128:(g + 1) * 128] = blk.T.astype(bf16)
            for j in range(F // 128):
                blk = gated(w1_ref[:, j * 128:(j + 1) * 128].astype(f32), 4 + j)
                w1t_ref[j * 128:(j + 1) * 128, :] = blk.T.astype(bf16)

        def load_q(j):
            return qt_ref[j // H, pl.ds(pl.multiple_of((j % H) * HP, HP), HP), :]

        def stage_pv(j, p_ref, hook=None):
            acc = jnp.zeros((HP, T), f32)
            for c0 in range(0, S, CK):
                p = pltpu.bitcast(p_ref[c0 // 2:(c0 + CK) // 2, :], bf16)
                part = _dot(vt_ref[c0 // T, :, c0 % T:c0 % T + CK], p)
                if hook is not None:
                    hook(c0, part)
                acc = acc + part
            o = acc * (1.0 / acc[DH:DH + 1, :])
            ot_ref[j // H, pl.ds(pl.multiple_of((j % H) * HP, HP), HP), :] = o.astype(bf16)

        def attention_exact(extra):
            if extra is not None:
                extra(lambda i, n: None)

            def body(j, c):
                q = load_q(j)
                row = lax.broadcasted_iota(jnp.int32, (HP, T), 0)
                q = jnp.where(row == DH, jnp.zeros_like(q), q)
                s = _dot(pltpu.bitcast(k_ref[...], bf16), q)
                s_ref[...] = s
                m = jnp.max(s, axis=0, keepdims=True)
                for c0 in range(0, S, CB):
                    p = jnp.exp2(s_ref[c0:c0 + CB, :] - m).astype(bf16)
                    plast_ref[c0 // 2:(c0 + CB) // 2, :] = pltpu.bitcast(p, u32)

                @pl.when(j < NJ - 1)
                def _():
                    stage_pv(j, plast_ref)
                return c
            lax.fori_loop(0, NJ, body, 0)

        def step(nkmax, ja, pa_ref, jc, pc_ref, vpu=True, extra=None):
            row = lax.broadcasted_iota(jnp.int32, (HP, T), 0)
            qf = load_q(ja).astype(f32)
            q = jnp.where(row == DH, qf * nkmax, qf).astype(bf16)
            sm = SM if vpu else S
            s = _dot(pltpu.bitcast(k_ref[0:sm // 2, :], bf16), q)
            pa_ref[0:sm // 2, :] = pltpu.bitcast(jnp.exp2(s).astype(bf16), u32)
            if extra is not None:
                extra(lambda i, n: s[((i * (sm // 8)) // n) * 8:((i * (sm // 8)) // n) * 8 + 8, 0:128])
            late = []
            if vpu:
                qf = q.astype(f32)
                for d in range(DH + 1):
                    qb_ref[d] = jnp.broadcast_to(qf[d:d + 1, :], (8, T))
                false = false_ref[...] != 0

                def chain(ci, tokens):
                    l, g = ci // NG, ci % NG
                    acc = None
                    for i, d in enumerate([DH] + list(range(DH))):
                        qr = qb_ref[d, :, l * 128:(l + 1) * 128]
                        if i % TS == 0:
                            qr = jnp.where(false, tokens(i), qr)
                        qr = jnp.concatenate([qr] * KT, axis=0)
                        if d == DH:
                            acc = qr
                        else:
                            acc = acc + kb_ref[d, g * 8 * KT:(g + 1) * 8 * KT, :] * qr
                    r0 = SM + g * 8 * KT
                    pa_ref[r0 // 2:(r0 + 8 * KT) // 2, l * 128:(l + 1) * 128] = pltpu.bitcast(
                        jnp.exp2(acc).astype(bf16), u32)

                na = int(round(NCH * FA))
                for ci in range(na):
                    def tokens(i, ci=ci):
                        n = ci * (DH + 1) + i
                        r = (n * (SM // 8)) // (na * (DH + 1))
                        l = ci // NG
                        return s[r * 8:(r + 1) * 8, l * 128:(l + 1) * 128]
                    chain(ci, tokens)
                late = list(range(na, NCH))
            if jc is not None:
                parts = {}
                stage_pv(jc, pc_ref, lambda c0, part: parts.__setitem__(c0 // CK, part))
                nsteps = len(late) * (DH + 1)
                per = (HP // 8) * NL
                for k, ci in enumerate(late):
                    def tokens(i, k=k):
                        pos = ((k * (DH + 1) + i) * (S // CK) * per) // nsteps
                        t, rem = pos // per, pos % per
                        r, l = rem // NL, rem % NL
                        return parts[t][r * 8:(r + 1) * 8, l * 128:(l + 1) * 128]
                    chain(ci, tokens)

        def attention_bounded(kmax, extra):
            nkmax = -kmax
            kf = pltpu.bitcast(k_ref[SM // 2:S // 2, :], bf16).astype(f32)
            for d in range(DH):
                kb_ref[d] = jnp.broadcast_to(kf[:, d:d + 1], (NVK, 128))
            step(nkmax, 0, p0_ref, None, None, vpu=False, extra=extra)
            assert UN % NP == 0
            nit = (NJ - 1) // UN

            def body(jj, c):
                j = UN * jj
                for u in range(UN):
                    step(nkmax, j + u + 1, P[(u + 1) % NP], j + u, P[u % NP])
                return c
            lax.fori_loop(0, nit, body, 0)
            for j in range(nit * UN, NJ - 1):
                step(nkmax, j + 1, P[(j + 1) % NP], j, P[j % NP])

        def attention(extra=None):
            nr = nrm_ref[...]
            qmax = jnp.max(nr[:, 0:1, :])
            kmax = jnp.sqrt(jnp.max(nr[:, 1:2, :])) * 1.01
            safe = qmax * kmax <= SAFE_BOUND
            if force == 'fast':
                attention_bounded(kmax, extra)
            elif force == 'safe':
                attention_exact(extra)
            else:
                lax.cond(safe, lambda: attention_bounded(kmax, extra), lambda: attention_exact(extra))
            stage_pv(NJ - 1, plast_ref)

        def out_cp(b):
            return pltpu.make_async_copy(xout_ref.at[b], o_hbm.at[:, pl.ds(pl.multiple_of(b * T, T), T)],
                                         sem_out.at[b])

        def post(layer):
            def body(b, carry):
                x = xt_ref[b] + _dot(wot_ref[...], ot_ref[b])
                ln = _ln_t(x)
                ht_ref[...] = jnp.maximum(_dot(w1t_ref[...], ln), 0.0).astype(bf16)
                x = x + _dot(w2t_ref[...], ht_ref[...])
                if layer == 0:
                    xt_ref[b] = x
                    qkv_post(b, qkv_mm(x))
                else:
                    xout_ref[b] = x.astype(bf16)
                    out_cp(b).start()
                return carry
            lax.fori_loop(0, NB, body, 0)

        w_cp[3].wait(); w_cp[4].wait(); w_cp[5].wait()
        attention(prep_post_weights)
        post(0)
        attention()
        post(1)
        for b in range(NB):
            out_cp(b).wait()

    scratch = [
        pltpu.VMEM((NB, D, T), bf16),
        pltpu.VMEM((D, D), bf16),
        pltpu.VMEM((DH, D), bf16),
        pltpu.VMEM((DH, D), bf16),
        pltpu.VMEM((D, D), bf16),
        pltpu.VMEM((D, F), bf16),
        pltpu.VMEM((D, F), bf16),
        pltpu.VMEM((NB, D, T), bf16),
        pltpu.VMEM((NB, D, T), f32),
        pltpu.VMEM((NB, H * HP, T), bf16),
        pltpu.VMEM((NB, H * HP, T), bf16),
        pltpu.VMEM((S // 2, HP), u32),
        pltpu.VMEM((NB, HP, T), bf16),
        pltpu.VMEM((S, T), f32),
        pltpu.VMEM((S // 2, T), u32),
        pltpu.VMEM((S // 2, T), u32),
        pltpu.VMEM((S // 2, T), u32),
        pltpu.VMEM((F, T), bf16),
        pltpu.VMEM((D + 2 * HP, D), bf16),
        pltpu.VMEM((D, H * HP), bf16),
        pltpu.VMEM((F, D), bf16),
        pltpu.VMEM((DH, NVK, 128), f32),
        pltpu.VMEM((DH + 1, 8, T), f32),
        pltpu.VMEM((NB, 2, T), f32),
        pltpu.VMEM((8, 128), jnp.int32),
        pltpu.SemaphoreType.DMA((NB,)),
        pltpu.SemaphoreType.DMA((6,)),
        pltpu.SemaphoreType.DMA((NB,)),
    ]
    return kernel, scratch


_KERNEL, _SCRATCH = make_kernel()


@jax.jit
def pallas_interleave_layers__grouped_kv_mqa__dense_activation_relu__prompt_kernel(
    A_x: jax.Array,
    A_wq: jax.Array,
    A_wk: jax.Array,
    A_wv: jax.Array,
    A_wo: jax.Array,
    B_x: jax.Array,
    B_w1: jax.Array,
    B_w2: jax.Array,
):
    del B_x
    out = pl.pallas_call(
        _KERNEL,
        out_shape=jax.ShapeDtypeStruct((D, S), bf16),
        in_specs=[pl.BlockSpec(memory_space=pl.ANY)] * 7,
        out_specs=pl.BlockSpec(memory_space=pl.ANY),
        scratch_shapes=_SCRATCH,
        compiler_params=pltpu.CompilerParams(vmem_limit_bytes=100 * 1024 * 1024),
    )(A_x.reshape(S, D).T, A_wq, A_wk.T, A_wv.T, A_wo, B_w1, B_w2.T)
    return out.T.reshape(1, S, D)
```
